```python
import os as _os
_os.environ.setdefault("JAX_PLATFORMS", "cpu")
import jax
import jax.numpy as jnp

def _softmax(x, axis=-1):
    return jax.nn.softmax(x, axis=axis)
def _gelu(x):
    return jax.nn.gelu(x, approximate=True)
def _silu(x):
    return jax.nn.silu(x)
def _sigmoid(x):
    return jax.nn.sigmoid(x)
def _layernorm(x, axis=-1, eps=1e-5):
    m = jnp.mean(x, axis=axis, keepdims=True)
    v = jnp.var(x, axis=axis, keepdims=True)
    return (x - m) / jnp.sqrt(v + eps)
def _scatter_add(tgt, idx, src, axis=0):
    return tgt.at[idx].add(src)
def _segment_sum(src, seg, n):
    return jax.ops.segment_sum(src, seg, n)
class _Rng:
    def __init__(self, key):
        self._k = key
    def _next(self):
        self._k, sub = jax.random.split(self._k)
        return sub
    def normal(self, shape):
        return jax.random.normal(self._next(), shape, dtype=jnp.bfloat16)
    def randint(self, lo, hi, shape):
        return jax.random.randint(self._next(), shape, lo, hi, dtype=jnp.int32)
    def uniform(self, shape, lo=0.0, hi=1.0):
        return jax.random.uniform(self._next(), shape, jnp.bfloat16, lo, hi)
    def permutation(self, n):
        return jax.random.permutation(self._next(), n)


kernel_name = 'recurrent_scan__ssm_conv_s5__mixer_s_mlp__prompt'

def setup_inputs():
    _rng = _Rng(jax.random.key(int.from_bytes(__import__("os").urandom(4), "little")))
    _w = (lambda a: (lambda t: t.astype(jnp.bfloat16) if jnp.issubdtype(t.dtype, jnp.floating) else t)(jnp.asarray(a)))
    def _A_setup():
        B, S, D = 1, 2048, 640
        P = D
        Lambda_re = -0.5 * jnp.exp((lambda *s: _rng.normal(s) * 0.8)(P))
        Lambda_im = (lambda *s: _rng.normal(s) * 0.8)(P) * 1.0
        B_re = (lambda *s: _rng.normal(s) * 0.8)(P, D) * (D ** -0.5)
        B_im = (lambda *s: _rng.normal(s) * 0.8)(P, D) * (D ** -0.5)
        C_re = (lambda *s: _rng.normal(s) * 0.8)(D, P) * (P ** -0.5)
        C_im = (lambda *s: _rng.normal(s) * 0.8)(D, P) * (P ** -0.5)
        log_dt = (lambda *s: _rng.normal(s) * 0.8)(P) * 0.3 - 2.0
        Dskip = (lambda *s: _rng.normal(s) * 0.8)(D)
        return {
            "x": _w((lambda *s: _rng.normal(s) * 0.05)(B, S, D)),
            "Lambda_re": _w(Lambda_re),
            "Lambda_im": _w(Lambda_im),
            "B_re": _w(B_re),
            "B_im": _w(B_im),
            "C_re": _w(C_re),
            "C_im": _w(C_im),
            "log_dt": _w(log_dt),
            "Dskip": _w(Dskip),
        }
    _A_in = _A_setup()

    def _B_setup():
        B, S, D, F = 1, 2048, 640, 1536
        return {
            "x":  _w((lambda *s: _rng.normal(s) * 0.05)(B, S, D)),
            "w1": _w((lambda *s: _rng.normal(s) * 0.8)(D, D) * (D ** -0.5)),
            "w2": _w((lambda *s: _rng.normal(s) * 0.8)(D, D) * (D ** -0.5)),
            "w3": _w((lambda *s: _rng.normal(s) * 0.8)(D, F) * (D ** -0.5)),
            "w4": _w((lambda *s: _rng.normal(s) * 0.8)(F, D) * (F ** -0.5)),
        }
    _B_in = _B_setup()

    return {
        "A_x": _A_in["x"],
        "A_Lambda_re": _A_in["Lambda_re"],
        "A_Lambda_im": _A_in["Lambda_im"],
        "A_B_re": _A_in["B_re"],
        "A_B_im": _A_in["B_im"],
        "A_C_re": _A_in["C_re"],
        "A_C_im": _A_in["C_im"],
        "A_log_dt": _A_in["log_dt"],
        "A_Dskip": _A_in["Dskip"],
        "B_x": _B_in["x"],
        "B_w1": _B_in["w1"],
        "B_w2": _B_in["w2"],
        "B_w3": _B_in["w3"],
        "B_w4": _B_in["w4"],
    }

def reference(A_x, A_Lambda_re, A_Lambda_im, A_B_re, A_B_im, A_C_re, A_C_im, A_log_dt, A_Dskip, B_x, B_w1, B_w2, B_w3, B_w4):
    def _A_ref(x, Lambda_re, Lambda_im, B_re, B_im, C_re, C_im, log_dt, Dskip):
        Bsz, L, H = x.shape
        Lam = Lambda_re + 1j * Lambda_im
        Bmat = B_re + 1j * B_im
        Cmat = C_re + 1j * C_im
        dt = jnp.exp(log_dt)
        Lam_bar = jnp.exp(dt * Lam)
        B_bar = ((Lam_bar - 1.0) / Lam)[:, None] * Bmat
        Bu = jnp.einsum("bld,pd->blp", x + 0j, B_bar)
        h = jnp.zeros_like(Bu[:, 0, :])
        hs = []
        for t in range(L):
            h = Lam_bar[None, :] * h + Bu[:, t, :]
            hs.append(h)
        hseq = jnp.stack(hs, 1)
        y = 2.0 * jnp.einsum("blp,dp->bld", hseq, Cmat).real + x * Dskip[None, None, :]
        return y

    def _B_ref(x, w1, w2, w3, w4):
        B, S, D = x.shape
        h = _gelu(_layernorm(x, axis=-1) @ w1)
        c = D // 4
        g0 = jnp.pad(h[:, :, 0*c:1*c], ((0, 0), (1, 0), (0, 0)))[:, :S, :]
        g1 = jnp.pad(h[:, :, 1*c:2*c], ((0, 0), (0, 1), (0, 0)))[:, 1:, :]
        g2 = jnp.pad(h[:, :, 2*c:3*c], ((0, 0), (2, 0), (0, 0)))[:, :S, :]
        g3 = jnp.pad(h[:, :, 3*c:   ], ((0, 0), (0, 2), (0, 0)))[:, 2:, :]
        hs = jnp.concatenate([g0, g1, g2, g3], axis=-1) @ w2
        x1 = x + hs
        h2 = _gelu(_layernorm(x1, axis=-1) @ w3) @ w4
        return x1 + h2

    x = A_x
    xn = _layernorm(x, axis=-1)
    s = _A_ref(xn, A_Lambda_re, A_Lambda_im, A_B_re, A_B_im, A_C_re, A_C_im, A_log_dt, A_Dskip)
    g = _silu(_B_ref(xn, B_w1, B_w2, B_w3, B_w4))
    return x + s * g
```

```python
import functools
import jax
import jax.numpy as jnp
from jax import lax
import jax.experimental.pallas as pl
import jax.experimental.pallas.tpu as pltpu

L, D, P, F = 2048, 640, 640, 1536
TM = 256
NB = L // TM
S = TM // 8 + 1
SL = TM - 7 * S
UR = 8 * S
HALO = 8
NT = P // 128
f32 = jnp.float32
bf16 = jnp.bfloat16


def _ln(x):
    m = jnp.mean(x, axis=-1, keepdims=True)
    xc = x - m
    v = jnp.mean(xc * xc, axis=-1, keepdims=True)
    return xc * lax.rsqrt(v + 1e-5)


def _gelu(x):
    c = 0.7978845608028654
    return 0.5 * x * (1.0 + jnp.tanh(c * (x + 0.044715 * (x * x * x))))


def _dot(a, b):
    return jnp.dot(a, b, preferred_element_type=f32)


def _dot_nt(a, b):
    return lax.dot_general(a, b, (((1,), (1,)), ((), ())), preferred_element_type=f32)


def _kernel(xa_ref, xd_ref, lre_ref, lim_ref, ldt_ref, dsk_ref,
            bre_hbm, bim_hbm, cre_hbm, cim_hbm, w1_hbm, w2_hbm, w3_hbm, w4_hbm,
            o_ref,
            cc_ref, lam_ref, carry_ref, u_ref, h_ref, win_ref, xn_ref, s_ref,
            bre_ref, bim_ref, cre_ref, cim_ref, w1_ref, w2_ref, w3_ref, w4_ref, sems):
    i = pl.program_id(0)
    _src = (w1_hbm, bre_hbm, bim_hbm, cre_hbm, cim_hbm, w2_hbm, w3_hbm, w4_hbm)
    _dst = (w1_ref, bre_ref, bim_ref, cre_ref, cim_ref, w2_ref, w3_ref, w4_ref)

    def cp(n):
        return pltpu.make_async_copy(_src[n], _dst[n], sems.at[n])
    slot = i % 3
    pslot = (i + 2) % 3
    dslot = (i + 1) % 3

    def init():
        lre = lre_ref[...].reshape(1, P).astype(f32)
        lim = lim_ref[...].reshape(1, P).astype(f32)
        dt = jnp.exp(ldt_ref[...].reshape(1, P).astype(f32)).astype(bf16).astype(f32)
        e = jnp.exp(dt * lre)
        zi = dt * lim
        lbr = e * jnp.cos(zi)
        lbi = e * jnp.sin(zi)
        nr = lbr - 1.0
        ni = lbi
        den = lre * lre + lim * lim
        cr = (nr * lre + ni * lim) / den
        ci = (ni * lre - nr * lim) / den
        lam_ref[0] = jnp.broadcast_to(lbr, (8, P))
        lam_ref[1] = jnp.broadcast_to(lbi, (8, P))
        br, bi = lbr, lbi
        pr = pi = None
        n = S
        while n:
            if n & 1:
                if pr is None:
                    pr, pi = br, bi
                else:
                    pr, pi = pr * br - pi * bi, pr * bi + pi * br
            n >>= 1
            if n:
                br, bi = br * br - bi * bi, 2.0 * br * bi
        for k in range(3):
            lam_ref[2 + 2 * k] = jnp.broadcast_to(pr, (8, P))
            lam_ref[3 + 2 * k] = jnp.broadcast_to(pi, (8, P))
            pr, pi = pr * pr - pi * pi, 2.0 * pr * pi
        carry_ref[...] = jnp.zeros_like(carry_ref)
        win_ref[0, 0:HALO, :] = jnp.zeros((HALO, D), f32)
        u_ref[:, TM:UR, :] = jnp.zeros((2 * NT, UR - TM, 128), f32)
        return cr, ci

    def init_cc(cr, ci):
        cre = cre_ref[...].astype(f32)
        cim = cim_ref[...].astype(f32)
        cc_ref[:, 0:P] = (2.0 * (cre * cr - cim * ci)).astype(bf16)
        cc_ref[:, P:2 * P] = (-2.0 * (cre * ci + cim * cr)).astype(bf16)

    def a_ln1():
        x = xa_ref[...].astype(f32)
        xn_b = _ln(x).astype(bf16)
        xn_ref[slot] = xn_b
        return xn_b

    def a_ln2(xn_b):
        return _ln(xn_b.astype(f32)).astype(bf16)

    def a_u(xn_b):
        ur_all = _dot_nt(xn_b, bre_ref[...])
        ui_all = _dot_nt(xn_b, bim_ref[...])
        for k in range(NT):
            u_ref[k, 0:TM, :] = ur_all[:, 128 * k:128 * (k + 1)]
            u_ref[NT + k, 0:TM, :] = ui_all[:, 128 * k:128 * (k + 1)]

    def a_w1(l2, first):
        a = _gelu(_dot(l2, w1_ref[...]))
        win_ref[slot, HALO:HALO + TM, :] = a
        win_ref[slot, HALO + TM:2 * HALO + TM, :] = jnp.zeros((HALO, D), f32)
        if not first:
            win_ref[slot, 0:HALO, :] = win_ref[pslot, TM:TM + HALO, :]
            win_ref[pslot, HALO + TM:2 * HALO + TM, :] = a[0:HALO, :]

    def a_scan():
        row = lax.broadcasted_iota(jnp.int32, (8, 128), 0)
        is0 = row == 0
        lss = [slice(128 * k, 128 * (k + 1)) for k in range(NT)]
        lr = [lam_ref[0, :, ls] for ls in lss]
        li = [lam_ref[1, :, ls] for ls in lss]
        fr = [u_ref[k, pl.ds(0, 8, stride=S), :] for k in range(NT)]
        fi = [u_ref[NT + k, pl.ds(0, 8, stride=S), :] for k in range(NT)]
        for j in range(1, S):
            for k in range(NT):
                ur = u_ref[k, pl.ds(j, 8, stride=S), :]
                ui = u_ref[NT + k, pl.ds(j, 8, stride=S), :]
                fr[k], fi[k] = (lr[k] * fr[k] - li[k] * fi[k] + ur,
                                lr[k] * fi[k] + li[k] * fr[k] + ui)
        hr = [None] * NT
        hi = [None] * NT
        for k in range(NT):
            ls = lss[k]
            cr_ = carry_ref[0, :, ls]
            ci_ = carry_ref[1, :, ls]
            sr, si = lam_ref[2, :, ls], lam_ref[3, :, ls]
            gr = fr[k] + jnp.where(is0, sr * cr_ - si * ci_, 0.0)
            gi = fi[k] + jnp.where(is0, sr * ci_ + si * cr_, 0.0)
            for q, d in enumerate((1, 2, 4)):
                sr, si = lam_ref[2 + 2 * q, :, ls], lam_ref[3 + 2 * q, :, ls]
                rr = pltpu.roll(gr, d, 0)
                ri = pltpu.roll(gi, d, 0)
                m = row >= d
                gr, gi = (gr + jnp.where(m, sr * rr - si * ri, 0.0),
                          gi + jnp.where(m, sr * ri + si * rr, 0.0))
            hr[k] = jnp.where(is0, cr_, pltpu.roll(gr, 1, 0))
            hi[k] = jnp.where(is0, ci_, pltpu.roll(gi, 1, 0))
        for j in range(S):
            for k in range(NT):
                ur = u_ref[k, pl.ds(j, 8, stride=S), :]
                ui = u_ref[NT + k, pl.ds(j, 8, stride=S), :]
                hr[k], hi[k] = (lr[k] * hr[k] - li[k] * hi[k] + ur,
                                lr[k] * hi[k] + li[k] * hr[k] + ui)
                h_ref[k, pl.ds(j, 8, stride=S), :] = hr[k]
                h_ref[NT + k, pl.ds(j, 8, stride=S), :] = hi[k]
                if j == SL - 1:
                    carry_ref[0, :, lss[k]] = jnp.broadcast_to(hr[k][7:8, :], (8, 128))
                    carry_ref[1, :, lss[k]] = jnp.broadcast_to(hi[k][7:8, :], (8, 128))

    def a_y(xn_b):
        hcat = jnp.concatenate([h_ref[k, 0:TM, :].astype(bf16) for k in range(2 * NT)], axis=1)
        y = _dot_nt(hcat, cc_ref[...])
        s_ref[slot] = y + xn_b.astype(f32) * dsk_ref[...].reshape(1, D).astype(f32)

    def d_shift():
        lane = lax.broadcasted_iota(jnp.int32, (TM, 128), 1)
        def rd(off, t):
            return win_ref[dslot, HALO + off:HALO + off + TM, 128 * t:128 * (t + 1)]
        t0 = rd(-1, 0)
        t1 = jnp.where(lane < 32, rd(-1, 1), rd(1, 1))
        t2 = jnp.where(lane < 64, rd(1, 2), rd(-2, 2))
        t3 = jnp.where(lane < 96, rd(-2, 3), rd(2, 3))
        t4 = rd(2, 4)
        return jnp.concatenate([t0.astype(bf16), t1.astype(bf16), t2.astype(bf16),
                                t3.astype(bf16), t4.astype(bf16)], axis=1)

    def d_w2(sh):
        return xn_ref[dslot].astype(f32) + _dot(sh, w2_ref[...])

    def d_ln3(x1):
        return _ln(x1).astype(bf16)

    def d_w3(l3):
        return _gelu(_dot(l3, w3_ref[...])).astype(bf16)

    def d_w4(z, x1):
        return x1 + _dot(z, w4_ref[...])

    def d_out(t):
        g = t * jax.nn.sigmoid(t)
        o_ref[...] = xd_ref[...].astype(f32) + s_ref[dslot] * g

    def only_a(first):
        xn_b = a_ln1()
        l2 = a_ln2(xn_b)
        a_u(xn_b)
        a_w1(l2, first)
        a_scan()
        a_y(xn_b)

    def only_d():
        sh = d_shift()
        x1 = d_w2(sh)
        l3 = d_ln3(x1)
        z = d_w3(l3)
        t = d_w4(z, x1)
        d_out(t)

    def both():
        sh = d_shift()
        x1 = d_w2(sh)
        xn_b = a_ln1()
        l2 = a_ln2(xn_b)
        a_u(xn_b)
        l3 = d_ln3(x1)
        z = d_w3(l3)
        a_scan()
        a_w1(l2, False)
        t = d_w4(z, x1)
        d_out(t)
        a_y(xn_b)

    @pl.when(i == 0)
    def _():
        for n in range(8):
            cp(n).start()
        cr, ci = init()
        xn_b = a_ln1()
        l2 = a_ln2(xn_b)
        cp(0).wait()
        a_w1(l2, True)
        cp(1).wait()
        cp(2).wait()
        a_u(xn_b)
        a_scan()
        cp(3).wait()
        cp(4).wait()
        init_cc(cr, ci)
        a_y(xn_b)

    @pl.when(i == 1)
    def _():
        only_a(False)
        cp(5).wait()
        cp(6).wait()
        cp(7).wait()

    @pl.when(jnp.logical_and(i > 1, i < NB))
    def _():
        both()

    @pl.when(i >= NB)
    def _():
        only_d()


@jax.jit
def pallas_recurrent_scan__ssm_conv_s5__mixer_s_mlp__prompt_kernel(
    A_x, A_Lambda_re, A_Lambda_im, A_B_re, A_B_im, A_C_re, A_C_im, A_log_dt, A_Dskip,
    B_x, B_w1, B_w2, B_w3, B_w4,
):
    x2 = A_x.reshape(L, D)
    vec = lambda v: v
    v1 = pl.BlockSpec((P,), lambda i: (0,))
    full = lambda shp: pl.BlockSpec(shp, lambda i: (0, 0))
    out = pl.pallas_call(
        _kernel,
        grid=(NB + 2,),
        in_specs=[
            pl.BlockSpec((TM, D), lambda i: (jnp.minimum(i, NB - 1), 0)),
            pl.BlockSpec((TM, D), lambda i: (jnp.maximum(i - 2, 0), 0)),
            v1, v1, v1, v1,
        ] + [pl.BlockSpec(memory_space=pl.ANY)] * 8 + [
        ],
        out_specs=pl.BlockSpec((TM, D), lambda i: (jnp.maximum(i - 2, 0), 0)),
        out_shape=jax.ShapeDtypeStruct((L, D), f32),
        scratch_shapes=[
            pltpu.VMEM((D, 2 * P), bf16),
            pltpu.VMEM((8, 8, P), f32),
            pltpu.VMEM((2, 8, P), f32),
            pltpu.VMEM((2 * NT, UR, 128), f32),
            pltpu.VMEM((2 * NT, UR, 128), f32),
            pltpu.VMEM((3, TM + 2 * HALO, D), f32),
            pltpu.VMEM((3, TM, D), bf16),
            pltpu.VMEM((3, TM, D), f32),
            pltpu.VMEM((P, D), bf16), pltpu.VMEM((P, D), bf16),
            pltpu.VMEM((D, P), bf16), pltpu.VMEM((D, P), bf16),
            pltpu.VMEM((D, D), bf16), pltpu.VMEM((D, D), bf16),
            pltpu.VMEM((D, F), bf16), pltpu.VMEM((F, D), bf16),
            pltpu.SemaphoreType.DMA((8,)),
        ],
        compiler_params=pltpu.CompilerParams(
            dimension_semantics=("arbitrary",),
            vmem_limit_bytes=100 * 1024 * 1024,
        ),
    )(x2, x2, vec(A_Lambda_re), vec(A_Lambda_im), vec(A_log_dt), vec(A_Dskip),
      A_B_re, A_B_im, A_C_re, A_C_im, B_w1, B_w2, B_w3, B_w4)
    return out.reshape(1, L, D)
```

```python
import functools
import jax
import jax.numpy as jnp
from jax import lax
import jax.experimental.pallas as pl
import jax.experimental.pallas.tpu as pltpu

L, D, P, F = 2048, 640, 640, 1536
TM = 256
NB = L // TM
S = TM // 8 + 1
SL = TM - 7 * S
UR = 8 * S
HALO = 8
NT = P // 128
CH = 32
f32 = jnp.float32
bf16 = jnp.bfloat16


def _ln(x):
    m = jnp.mean(x, axis=-1, keepdims=True)
    xc = x - m
    v = jnp.mean(xc * xc, axis=-1, keepdims=True)
    return xc * lax.rsqrt(v + 1e-5)


def _gelu(x):
    c = 0.7978845608028654
    return 0.5 * x * (1.0 + jnp.tanh(c * (x + 0.044715 * (x * x * x))))


def _dot(a, b):
    return jnp.dot(a, b, preferred_element_type=f32)


def _dot_nt(a, b):
    return lax.dot_general(a, b, (((1,), (1,)), ((), ())), preferred_element_type=f32)


def _kernel(x_hbm, lre_hbm, lim_hbm, ldt_hbm, dsk_hbm,
            bre_hbm, bim_hbm, cre_hbm, cim_hbm, w1_hbm, w2_hbm, w3_hbm, w4_hbm,
            o_ref,
            cc_ref, lam_ref, carry_ref, u_ref, u2_ref, h_ref, win_ref, xn_ref, s_ref,
            bre_ref, bim_ref, cre_ref, cim_ref, w1_ref, w2_ref, w3_ref, w4_ref,
            x_ref, lre_ref, lim_ref, ldt_ref, dsk_ref, sems, xsems,
            l2_ref, l3_ref, x1_ref, h2_ref, o_scr, osems):
    st = pl.program_id(0)
    _src = (w1_hbm, bre_hbm, bim_hbm, cre_hbm, cim_hbm, w2_hbm, w3_hbm, w4_hbm,
            lre_hbm, lim_hbm, ldt_hbm, dsk_hbm)
    _dst = (w1_ref, bre_ref.at[0:P], bre_ref.at[P:2 * P], cre_ref, cim_ref, w2_ref, w3_ref, w4_ref,
            lre_ref, lim_ref, ldt_ref, dsk_ref)

    def cp(n):
        return pltpu.make_async_copy(_src[n], _dst[n], sems.at[n])

    def rows(b):
        if isinstance(b, int):
            return pl.ds(b * TM, TM)
        return pl.ds(pl.multiple_of(b * TM, TM), TM)

    def cpx(b):
        return pltpu.make_async_copy(x_hbm.at[rows(b)], x_ref.at[rows(b)], xsems.at[b])

    HM = TM // 2

    def cpo(b, hh):
        osl = b % 2
        return pltpu.make_async_copy(
            o_scr.at[osl, pl.ds(hh * HM, HM)],
            o_ref.at[pl.ds(pl.multiple_of(b * TM + hh * HM, HM), HM)],
            osems.at[osl * 2 + hh])

    def init():
        lre = lre_ref[...].reshape(1, P).astype(f32)
        lim = lim_ref[...].reshape(1, P).astype(f32)
        dt = jnp.exp(ldt_ref[...].reshape(1, P).astype(f32)).astype(bf16).astype(f32)
        e = jnp.exp(dt * lre)
        zi = dt * lim
        lbr = e * jnp.cos(zi)
        lbi = e * jnp.sin(zi)
        nr = lbr - 1.0
        ni = lbi
        den = lre * lre + lim * lim
        cr = (nr * lre + ni * lim) / den
        ci = (ni * lre - nr * lim) / den
        lam_ref[0] = jnp.broadcast_to(lbr, (8, P))
        lam_ref[1] = jnp.broadcast_to(lbi, (8, P))
        br, bi = lbr, lbi
        pr = pi = None
        n = S
        while n:
            if n & 1:
                if pr is None:
                    pr, pi = br, bi
                else:
                    pr, pi = pr * br - pi * bi, pr * bi + pi * br
            n >>= 1
            if n:
                br, bi = br * br - bi * bi, 2.0 * br * bi
        for k in range(3):
            lam_ref[2 + 2 * k] = jnp.broadcast_to(pr, (8, P))
            lam_ref[3 + 2 * k] = jnp.broadcast_to(pi, (8, P))
            pr, pi = pr * pr - pi * pi, 2.0 * pr * pi
        carry_ref[...] = jnp.zeros_like(carry_ref)
        win_ref[0, 0:HALO, :] = jnp.zeros((HALO, D), f32)
        u_ref[:, TM:UR, :] = jnp.zeros((2 * NT, UR - TM, 128), f32)
        u2_ref[:, TM:UR, :] = jnp.zeros((2 * NT, UR - TM, 128), f32)
        return cr, ci

    def init_cc(cr, ci):
        cre = cre_ref[...].astype(f32)
        cim = cim_ref[...].astype(f32)
        cc_ref[:, 0:P] = (2.0 * (cre * cr - cim * ci)).astype(bf16)
        cc_ref[:, P:2 * P] = (-2.0 * (cre * ci + cim * cr)).astype(bf16)

    def a_ln1(b, slot):
        for c in range(TM // CH):
            if isinstance(b, int):
                r = pl.ds(b * TM + c * CH, CH)
            else:
                r = pl.ds(pl.multiple_of(b * TM + c * CH, CH), CH)
            xn_c = _ln(x_ref[r, :].astype(f32)).astype(bf16)
            xn_ref[slot, c * CH:(c + 1) * CH, :] = xn_c
            l2_ref[c * CH:(c + 1) * CH, :] = _ln(xn_c.astype(f32)).astype(bf16)
        return xn_ref[slot]

    def a_ln2(xn_b):
        return l2_ref[...]

    def a_u(xn_b, ur_):
        u_all = _dot_nt(xn_b, bre_ref[...])
        for k in range(2 * NT):
            ur_[k, 0:TM, :] = u_all[:, 128 * k:128 * (k + 1)]

    def a_w1(l2, slot, pslot):
        a = _gelu(_dot(l2, w1_ref[...]))
        win_ref[slot, HALO:HALO + TM, :] = a
        win_ref[slot, HALO + TM:2 * HALO + TM, :] = jnp.zeros((HALO, D), f32)
        if pslot is not None:
            win_ref[slot, 0:HALO, :] = win_ref[pslot, TM:TM + HALO, :]
            win_ref[pslot, HALO + TM:2 * HALO + TM, :] = a[0:HALO, :]

    def a_scan(ur_, h_ref=h_ref):
        row = lax.broadcasted_iota(jnp.int32, (8, 128), 0)
        is0 = row == 0
        lss = [slice(128 * k, 128 * (k + 1)) for k in range(NT)]
        lr = [lam_ref[0, :, ls] for ls in lss]
        li = [lam_ref[1, :, ls] for ls in lss]
        fr = [ur_[k, pl.ds(0, 8, stride=S), :] for k in range(NT)]
        fi = [ur_[NT + k, pl.ds(0, 8, stride=S), :] for k in range(NT)]
        for j in range(1, S):
            for k in range(NT):
                ur = ur_[k, pl.ds(j, 8, stride=S), :]
                ui = ur_[NT + k, pl.ds(j, 8, stride=S), :]
                fr[k], fi[k] = (lr[k] * fr[k] - li[k] * fi[k] + ur,
                                lr[k] * fi[k] + li[k] * fr[k] + ui)
        hr = [None] * NT
        hi = [None] * NT
        for k in range(NT):
            ls = lss[k]
            cr_ = carry_ref[0, :, ls]
            ci_ = carry_ref[1, :, ls]
            sr, si = lam_ref[2, :, ls], lam_ref[3, :, ls]
            gr = fr[k] + jnp.where(is0, sr * cr_ - si * ci_, 0.0)
            gi = fi[k] + jnp.where(is0, sr * ci_ + si * cr_, 0.0)
            for q, d in enumerate((1, 2, 4)):
                sr, si = lam_ref[2 + 2 * q, :, ls], lam_ref[3 + 2 * q, :, ls]
                rr = pltpu.roll(gr, d, 0)
                ri = pltpu.roll(gi, d, 0)
                m = row >= d
                gr, gi = (gr + jnp.where(m, sr * rr - si * ri, 0.0),
                          gi + jnp.where(m, sr * ri + si * rr, 0.0))
            hr[k] = jnp.where(is0, cr_, pltpu.roll(gr, 1, 0))
            hi[k] = jnp.where(is0, ci_, pltpu.roll(gi, 1, 0))
        for j in range(S):
            for k in range(NT):
                ur = ur_[k, pl.ds(j, 8, stride=S), :]
                ui = ur_[NT + k, pl.ds(j, 8, stride=S), :]
                hr[k], hi[k] = (lr[k] * hr[k] - li[k] * hi[k] + ur,
                                lr[k] * hi[k] + li[k] * hr[k] + ui)
                h_ref[k, pl.ds(j, 8, stride=S), :] = hr[k]
                h_ref[NT + k, pl.ds(j, 8, stride=S), :] = hi[k]
                if j == SL - 1:
                    carry_ref[0, :, lss[k]] = jnp.broadcast_to(hr[k][7:8, :], (8, 128))
                    carry_ref[1, :, lss[k]] = jnp.broadcast_to(hi[k][7:8, :], (8, 128))

    def a_y(xn_b, slot, h_ref=h_ref):
        hcat = jnp.concatenate([h_ref[k, 0:TM, :].astype(bf16) for k in range(2 * NT)], axis=1)
        y = _dot_nt(hcat, cc_ref[...])
        s_ref[slot] = y + xn_b.astype(f32) * dsk_ref[...].reshape(1, D).astype(f32)

    def d_shift(dslot):
        lane = lax.broadcasted_iota(jnp.int32, (TM, 128), 1)
        def rd(off, t):
            return win_ref[dslot, HALO + off:HALO + off + TM, 128 * t:128 * (t + 1)]
        t0 = rd(-1, 0)
        t1 = jnp.where(lane < 32, rd(-1, 1), rd(1, 1))
        t2 = jnp.where(lane < 64, rd(1, 2), rd(-2, 2))
        t3 = jnp.where(lane < 96, rd(-2, 3), rd(2, 3))
        t4 = rd(2, 4)
        return jnp.concatenate([t0.astype(bf16), t1.astype(bf16), t2.astype(bf16),
                                t3.astype(bf16), t4.astype(bf16)], axis=1)

    def d_w2(sh, dslot):
        x1_ref[...] = xn_ref[dslot].astype(f32) + _dot(sh, w2_ref[...])
        return None

    def d_ln3(x1):
        for c in range(TM // CH):
            l3_ref[c * CH:(c + 1) * CH, :] = _ln(x1_ref[c * CH:(c + 1) * CH, :]).astype(bf16)
        return l3_ref[...]

    def d_w3(l3):
        return _gelu(_dot(l3, w3_ref[...])).astype(bf16)

    def d_w4(z, x1):
        return x1_ref[...] + _dot(z, w4_ref[...])

    def d_out(t, b, dslot):
        g = t * jax.nn.sigmoid(t)
        o_scr[b % 2] = x_ref[rows(b), :].astype(f32) + s_ref[dslot] * g
        cpo(b, 0).start()
        cpo(b, 1).start()

    @pl.when(st == 0)
    def _():
        cpx(0).start()
        for n in (8, 9, 10, 11):
            cp(n).start()
        cp(0).start()
        cpx(1).start()
        for n in (1, 2, 3, 4):
            cp(n).start()
        cpx(2).start()
        for n in (5, 6, 7):
            cp(n).start()
        for b in range(3, NB):
            cpx(b).start()
        cpx(0).wait()
        xn0 = a_ln1(0, 0)
        l20 = a_ln2(xn0)
        for n in (8, 9, 10, 11):
            cp(n).wait()
        cpx(1).wait()
        cp(0).wait()
        a_w1(l20, 0, None)
        cr, ci = init()
        xn1 = a_ln1(1, 1)
        l21 = a_ln2(xn1)
        a_w1(l21, 1, 0)
        cp(1).wait()
        cp(2).wait()
        a_u(xn0, u_ref)
        a_scan(u_ref)
        a_u(xn1, u2_ref)
        cp(3).wait()
        cp(4).wait()
        cpx(2).wait()
        init_cc(cr, ci)
        a_scan(u2_ref, h2_ref)
        a_y(xn0, 0)
        a_ln1(2, 2)
        a_y(xn1, 1, h2_ref)
        cp(5).wait()
        cp(6).wait()
        cp(7).wait()

    @pl.when(st >= 3)
    def _():
        cpo(st - 3, 0).wait()
        cpo(st - 3, 1).wait()

    def mid(ahead):
        b = st + 1
        slot = b % 3
        pslot = st % 3
        dslot = (st + 2) % 3
        if ahead:
            cpx(b + 1).wait()
        sh = d_shift(dslot)
        x1 = d_w2(sh, (st + 3) % 4)
        xn_b = xn_ref[b % 4]
        a_u(xn_b, u_ref)
        l3 = d_ln3(x1)
        z = d_w3(l3)
        a_scan(u_ref)
        a_w1(l2_ref[...], slot, pslot)
        t = d_w4(z, x1)
        d_out(t, st - 1, dslot)
        if ahead:
            a_ln1(b + 1, (b + 1) % 4)
        a_y(xn_b, slot)

    @pl.when(jnp.logical_and(st > 0, st < NB - 2))
    def _():
        mid(True)

    @pl.when(st == NB - 2)
    def _():
        mid(False)

    @pl.when(st >= NB - 1)
    def _():
        dslot = (st + 2) % 3
        xslot = (st + 3) % 4
        lane = lax.broadcasted_iota(jnp.int32, (HM, 128), 1)
        x1s = []
        for hh in range(2):
            r0 = hh * HM
            def rd(off, t):
                return win_ref[dslot, HALO + r0 + off:HALO + r0 + off + HM, 128 * t:128 * (t + 1)]
            t0 = rd(-1, 0)
            t1 = jnp.where(lane < 32, rd(-1, 1), rd(1, 1))
            t2 = jnp.where(lane < 64, rd(1, 2), rd(-2, 2))
            t3 = jnp.where(lane < 96, rd(-2, 3), rd(2, 3))
            t4 = rd(2, 4)
            sh = jnp.concatenate([t0.astype(bf16), t1.astype(bf16), t2.astype(bf16),
                                  t3.astype(bf16), t4.astype(bf16)], axis=1)
            x1s.append(xn_ref[xslot, r0:r0 + HM, :].astype(f32) + _dot(sh, w2_ref[...]))
        zs = []
        for hh in range(2):
            l3 = _ln(x1s[hh]).astype(bf16)
            zs.append(_gelu(_dot(l3, w3_ref[...])).astype(bf16))
        for hh in range(2):
            r0 = hh * HM
            t = x1s[hh] + _dot(zs[hh], w4_ref[...])
            g = t * jax.nn.sigmoid(t)
            xr = pl.ds(pl.multiple_of((st - 1) * TM + r0, HM), HM)
            o_scr[(st - 1) % 2, r0:r0 + HM, :] = x_ref[xr, :].astype(f32) + s_ref[dslot, r0:r0 + HM, :] * g
            cpo(st - 1, hh).start()

    @pl.when(st == NB)
    def _():
        for b in (NB - 2, NB - 1):
            cpo(b, 0).wait()
            cpo(b, 1).wait()


@jax.jit
def pallas_recurrent_scan__ssm_conv_s5__mixer_s_mlp__prompt_kernel(
    A_x, A_Lambda_re, A_Lambda_im, A_B_re, A_B_im, A_C_re, A_C_im, A_log_dt, A_Dskip,
    B_x, B_w1, B_w2, B_w3, B_w4,
):
    x2 = A_x.reshape(L, D)
    out = pl.pallas_call(
        _kernel,
        grid=(NB + 1,),
        in_specs=[pl.BlockSpec(memory_space=pl.ANY)] * 13,
        out_specs=pl.BlockSpec(memory_space=pl.ANY),
        out_shape=jax.ShapeDtypeStruct((L, D), f32),
        scratch_shapes=[
            pltpu.VMEM((D, 2 * P), bf16),
            pltpu.VMEM((8, 8, P), f32),
            pltpu.VMEM((2, 8, P), f32),
            pltpu.VMEM((2 * NT, UR, 128), f32),
            pltpu.VMEM((2 * NT, UR, 128), f32),
            pltpu.VMEM((2 * NT, UR, 128), f32),
            pltpu.VMEM((3, TM + 2 * HALO, D), f32),
            pltpu.VMEM((4, TM, D), bf16),
            pltpu.VMEM((3, TM, D), f32),
            pltpu.VMEM((2 * P, D), bf16), pltpu.VMEM((8, 128), bf16),
            pltpu.VMEM((D, P), bf16), pltpu.VMEM((D, P), bf16),
            pltpu.VMEM((D, D), bf16), pltpu.VMEM((D, D), bf16),
            pltpu.VMEM((D, F), bf16), pltpu.VMEM((F, D), bf16),
            pltpu.VMEM((L, D), bf16),
            pltpu.VMEM((P,), bf16), pltpu.VMEM((P,), bf16),
            pltpu.VMEM((P,), bf16), pltpu.VMEM((D,), bf16),
            pltpu.SemaphoreType.DMA((12,)),
            pltpu.SemaphoreType.DMA((NB,)),
            pltpu.VMEM((TM, D), bf16), pltpu.VMEM((TM, D), bf16), pltpu.VMEM((TM, D), f32),
            pltpu.VMEM((2 * NT, UR, 128), f32),
            pltpu.VMEM((2, TM, D), f32),
            pltpu.SemaphoreType.DMA((4,)),
        ],
        compiler_params=pltpu.CompilerParams(
            dimension_semantics=("arbitrary",),
            vmem_limit_bytes=100 * 1024 * 1024,
        ),
    )(x2, A_Lambda_re, A_Lambda_im, A_log_dt, A_Dskip,
      A_B_re, A_B_im, A_C_re, A_C_im, B_w1, B_w2, B_w3, B_w4)
    return out.reshape(1, L, D)
```

```python
import jax
import jax.numpy as jnp
from jax import lax
import jax.experimental.pallas as pl
import jax.experimental.pallas.tpu as pltpu

L, D, P, F = 2048, 640, 640, 1536
TM = 256
NB = L // TM
HM = TM // 2
S = TM // 8 + 1
SL = TM - 7 * S
UR = 8 * S
HALO = 8
NT = P // 128
CH = 8
f32 = jnp.float32
bf16 = jnp.bfloat16


def _ln(x):
    m = jnp.mean(x, axis=-1, keepdims=True)
    xc = x - m
    v = jnp.mean(xc * xc, axis=-1, keepdims=True)
    return xc * lax.rsqrt(v + 1e-5)


def _gelu(x):
    c = 0.7978845608028654
    return 0.5 * x * (1.0 + jnp.tanh(c * (x + 0.044715 * (x * x * x))))


def _dot(a, b):
    return jnp.dot(a, b, preferred_element_type=f32)


def _dot_nt(a, b):
    return lax.dot_general(a, b, (((1,), (1,)), ((), ())), preferred_element_type=f32)


def _kernel(x_hbm, lre_hbm, lim_hbm, ldt_hbm, dsk_hbm,
            bre_hbm, bim_hbm, cre_hbm, cim_hbm, w1_hbm, w2_hbm, w3_hbm, w4_hbm,
            o_ref,
            cc_ref, lam_ref, carry_ref, u_ref, u2_ref, h_ref, win_ref, xn_ref, s_ref,
            bre_ref, cre_ref, cim_ref, w1_ref, w2_ref, w3_ref, w4_ref,
            x_ref, lre_ref, lim_ref, ldt_ref, dsk_ref, sems, xsems,
            l2_ref, l3_ref, x1_ref, h2_ref, o_scr, osems):
    st = pl.program_id(0)
    _src = (w1_hbm, bre_hbm, bim_hbm, cre_hbm, cim_hbm, w2_hbm, w3_hbm, w4_hbm,
            lre_hbm, lim_hbm, ldt_hbm, dsk_hbm)
    _dst = (w1_ref, bre_ref.at[0:P], bre_ref.at[P:2 * P], cre_ref, cim_ref, w2_ref, w3_ref, w4_ref,
            lre_ref, lim_ref, ldt_ref, dsk_ref)

    def cp(n):
        return pltpu.make_async_copy(_src[n], _dst[n], sems.at[n])

    def rows(b):
        if isinstance(b, int):
            return pl.ds(b * TM, TM)
        return pl.ds(pl.multiple_of(b * TM, TM), TM)

    def cpx(b):
        return pltpu.make_async_copy(x_hbm.at[rows(b)], x_ref.at[rows(b)], xsems.at[b])

    def cpo(b, hh):
        osl = b % 2
        return pltpu.make_async_copy(
            o_scr.at[osl, pl.ds(hh * HM, HM)],
            o_ref.at[pl.ds(pl.multiple_of(b * TM + hh * HM, HM), HM)],
            osems.at[osl * 2 + hh])

    def init():
        lre = lre_ref[...].reshape(1, P).astype(f32)
        lim = lim_ref[...].reshape(1, P).astype(f32)
        dt = jnp.exp(ldt_ref[...].reshape(1, P).astype(f32)).astype(bf16).astype(f32)
        e = jnp.exp(dt * lre)
        zi = dt * lim
        lbr = e * jnp.cos(zi)
        lbi = e * jnp.sin(zi)
        nr = lbr - 1.0
        ni = lbi
        den = lre * lre + lim * lim
        cr = (nr * lre + ni * lim) / den
        ci = (ni * lre - nr * lim) / den
        lam_ref[0] = jnp.broadcast_to(lbr, (8, P))
        lam_ref[1] = jnp.broadcast_to(lbi, (8, P))
        br, bi = lbr, lbi
        pr = pi = None
        n = S
        while n:
            if n & 1:
                if pr is None:
                    pr, pi = br, bi
                else:
                    pr, pi = pr * br - pi * bi, pr * bi + pi * br
            n >>= 1
            if n:
                br, bi = br * br - bi * bi, 2.0 * br * bi
        for k in range(3):
            lam_ref[2 + 2 * k] = jnp.broadcast_to(pr, (8, P))
            lam_ref[3 + 2 * k] = jnp.broadcast_to(pi, (8, P))
            pr, pi = pr * pr - pi * pi, 2.0 * pr * pi
        carry_ref[...] = jnp.zeros_like(carry_ref)
        win_ref[0, 0:HALO, :] = jnp.zeros((HALO, D), f32)
        u_ref[:, TM:UR, :] = jnp.zeros((2 * NT, UR - TM, 128), f32)
        u2_ref[:, TM:UR, :] = jnp.zeros((2 * NT, UR - TM, 128), f32)
        return cr, ci

    def init_cc(cr, ci):
        cre = cre_ref[...].astype(f32)
        cim = cim_ref[...].astype(f32)
        cc_ref[:, 0:P] = (2.0 * (cre * cr - cim * ci)).astype(bf16)
        cc_ref[:, P:2 * P] = (-2.0 * (cre * ci + cim * cr)).astype(bf16)

    def a_ln1(b, slot):
        for c in range(TM // CH):
            if isinstance(b, int):
                r = pl.ds(b * TM + c * CH, CH)
            else:
                r = pl.ds(pl.multiple_of(b * TM + c * CH, CH), CH)
            xn_c = _ln(x_ref[r, :].astype(f32)).astype(bf16)
            xn_ref[slot, c * CH:(c + 1) * CH, :] = xn_c
            l2_ref[c * CH:(c + 1) * CH, :] = _ln(xn_c.astype(f32)).astype(bf16)
        return xn_ref[slot]

    def a_u(xn_b, ur_):
        u_all = _dot_nt(xn_b, bre_ref[...])
        for k in range(2 * NT):
            ur_[k, 0:TM, :] = u_all[:, 128 * k:128 * (k + 1)]

    def a_w1(l2, slot, pslot):
        a = _gelu(_dot(l2, w1_ref[...]))
        win_ref[slot, HALO:HALO + TM, :] = a
        win_ref[slot, HALO + TM:2 * HALO + TM, :] = jnp.zeros((HALO, D), f32)
        if pslot is not None:
            win_ref[slot, 0:HALO, :] = win_ref[pslot, TM:TM + HALO, :]
            win_ref[pslot, HALO + TM:2 * HALO + TM, :] = a[0:HALO, :]

    def a_scan(ur_, h_ref=h_ref):
        row = lax.broadcasted_iota(jnp.int32, (8, 128), 0)
        is0 = row == 0
        lss = [slice(128 * k, 128 * (k + 1)) for k in range(NT)]
        lr = [lam_ref[0, :, ls] for ls in lss]
        li = [lam_ref[1, :, ls] for ls in lss]
        fr = [ur_[k, pl.ds(0, 8, stride=S), :] for k in range(NT)]
        fi = [ur_[NT + k, pl.ds(0, 8, stride=S), :] for k in range(NT)]
        for j in range(1, S):
            for k in range(NT):
                ur = ur_[k, pl.ds(j, 8, stride=S), :]
                ui = ur_[NT + k, pl.ds(j, 8, stride=S), :]
                fr[k], fi[k] = (lr[k] * fr[k] - li[k] * fi[k] + ur,
                                lr[k] * fi[k] + li[k] * fr[k] + ui)
        hr = [None] * NT
        hi = [None] * NT
        for k in range(NT):
            ls = lss[k]
            cr_ = carry_ref[0, :, ls]
            ci_ = carry_ref[1, :, ls]
            sr, si = lam_ref[2, :, ls], lam_ref[3, :, ls]
            gr = fr[k] + jnp.where(is0, sr * cr_ - si * ci_, 0.0)
            gi = fi[k] + jnp.where(is0, sr * ci_ + si * cr_, 0.0)
            for q, d in enumerate((1, 2, 4)):
                sr, si = lam_ref[2 + 2 * q, :, ls], lam_ref[3 + 2 * q, :, ls]
                rr = pltpu.roll(gr, d, 0)
                ri = pltpu.roll(gi, d, 0)
                m = row >= d
                gr, gi = (gr + jnp.where(m, sr * rr - si * ri, 0.0),
                          gi + jnp.where(m, sr * ri + si * rr, 0.0))
            hr[k] = jnp.where(is0, cr_, pltpu.roll(gr, 1, 0))
            hi[k] = jnp.where(is0, ci_, pltpu.roll(gi, 1, 0))
        for j in range(S):
            for k in range(NT):
                ur = ur_[k, pl.ds(j, 8, stride=S), :]
                ui = ur_[NT + k, pl.ds(j, 8, stride=S), :]
                hr[k], hi[k] = (lr[k] * hr[k] - li[k] * hi[k] + ur,
                                lr[k] * hi[k] + li[k] * hr[k] + ui)
                h_ref[k, pl.ds(j, 8, stride=S), :] = hr[k]
                h_ref[NT + k, pl.ds(j, 8, stride=S), :] = hi[k]
                if j == SL - 1:
                    carry_ref[0, :, lss[k]] = jnp.broadcast_to(hr[k][7:8, :], (8, 128))
                    carry_ref[1, :, lss[k]] = jnp.broadcast_to(hi[k][7:8, :], (8, 128))

    def a_y(xn_b, slot, h_ref=h_ref):
        hcat = jnp.concatenate([h_ref[k, 0:TM, :].astype(bf16) for k in range(2 * NT)], axis=1)
        y = _dot_nt(hcat, cc_ref[...])
        s_ref[slot] = y + xn_b.astype(f32) * dsk_ref[...].reshape(1, D).astype(f32)

    def d_shift(dslot, r0, n):
        lane = lax.broadcasted_iota(jnp.int32, (n, 128), 1)

        def rd(off, t):
            return win_ref[dslot, HALO + r0 + off:HALO + r0 + off + n, 128 * t:128 * (t + 1)]
        t0 = rd(-1, 0)
        t1 = jnp.where(lane < 32, rd(-1, 1), rd(1, 1))
        t2 = jnp.where(lane < 64, rd(1, 2), rd(-2, 2))
        t3 = jnp.where(lane < 96, rd(-2, 3), rd(2, 3))
        t4 = rd(2, 4)
        return jnp.concatenate([t0.astype(bf16), t1.astype(bf16), t2.astype(bf16),
                                t3.astype(bf16), t4.astype(bf16)], axis=1)

    def d_w2(sh, xslot):
        x1_ref[...] = xn_ref[xslot].astype(f32) + _dot(sh, w2_ref[...])

    def d_ln3():
        for c in range(TM // CH):
            l3_ref[c * CH:(c + 1) * CH, :] = _ln(x1_ref[c * CH:(c + 1) * CH, :]).astype(bf16)
        return l3_ref[...]

    def d_w3(l3):
        return _gelu(_dot(l3, w3_ref[...])).astype(bf16)

    def d_w4(z):
        return x1_ref[...] + _dot(z, w4_ref[...])

    def d_out(t, b, dslot):
        g = t * jax.nn.sigmoid(t)
        o_scr[b % 2] = x_ref[rows(b), :].astype(f32) + s_ref[dslot] * g
        cpo(b, 0).start()
        cpo(b, 1).start()

    @pl.when(st == 0)
    def _():
        cpx(0).start()
        for n in (8, 9, 10, 11):
            cp(n).start()
        cp(0).start()
        cpx(1).start()
        for n in (1, 2, 3, 4):
            cp(n).start()
        cpx(2).start()
        for n in (5, 6, 7):
            cp(n).start()
        for b in range(3, NB):
            cpx(b).start()
        cpx(0).wait()
        xn0 = a_ln1(0, 0)
        l20 = l2_ref[...]
        for n in (8, 9, 10, 11):
            cp(n).wait()
        cpx(1).wait()
        cp(0).wait()
        a_w1(l20, 0, None)
        cr, ci = init()
        xn1 = a_ln1(1, 1)
        l21 = l2_ref[...]
        a_w1(l21, 1, 0)
        cp(1).wait()
        cp(2).wait()
        a_u(xn0, u_ref)
        a_scan(u_ref)
        a_u(xn1, u2_ref)
        cp(3).wait()
        cp(4).wait()
        cpx(2).wait()
        init_cc(cr, ci)
        a_scan(u2_ref, h2_ref)
        a_y(xn0, 0)
        a_ln1(2, 2)
        a_y(xn1, 1, h2_ref)
        cp(5).wait()
        cp(6).wait()
        cp(7).wait()

    @pl.when(st >= 3)
    def _():
        cpo(st - 3, 0).wait()
        cpo(st - 3, 1).wait()

    def mid(ahead):
        b = st + 1
        slot = b % 3
        pslot = st % 3
        dslot = (st + 2) % 3
        if ahead:
            cpx(b + 1).wait()
        sh = d_shift(dslot, 0, TM)
        d_w2(sh, (st + 3) % 4)
        xn_b = xn_ref[b % 4]
        a_u(xn_b, u_ref)
        l3 = d_ln3()
        z = d_w3(l3)
        a_scan(u_ref)
        a_w1(l2_ref[...], slot, pslot)
        t = d_w4(z)
        d_out(t, st - 1, dslot)
        if ahead:
            a_ln1(b + 1, (b + 1) % 4)
        a_y(xn_b, slot)

    @pl.when(jnp.logical_and(st > 0, st < NB - 2))
    def _():
        mid(True)

    @pl.when(st == NB - 2)
    def _():
        mid(False)

    @pl.when(st >= NB - 1)
    def _():
        dslot = (st + 2) % 3
        xslot = (st + 3) % 4
        x1s = []
        for hh in range(2):
            r0 = hh * HM
            sh = d_shift(dslot, r0, HM)
            x1s.append(xn_ref[xslot, r0:r0 + HM, :].astype(f32) + _dot(sh, w2_ref[...]))
        zs = []
        for hh in range(2):
            l3 = _ln(x1s[hh]).astype(bf16)
            zs.append(_gelu(_dot(l3, w3_ref[...])).astype(bf16))
        for hh in range(2):
            r0 = hh * HM
            t = x1s[hh] + _dot(zs[hh], w4_ref[...])
            g = t * jax.nn.sigmoid(t)
            xr = pl.ds(pl.multiple_of((st - 1) * TM + r0, HM), HM)
            o_scr[(st - 1) % 2, r0:r0 + HM, :] = (
                x_ref[xr, :].astype(f32) + s_ref[dslot, r0:r0 + HM, :] * g)
            cpo(st - 1, hh).start()

    @pl.when(st == NB)
    def _():
        for b in (NB - 2, NB - 1):
            cpo(b, 0).wait()
            cpo(b, 1).wait()


@jax.jit
def pallas_recurrent_scan__ssm_conv_s5__mixer_s_mlp__prompt_kernel(
    A_x, A_Lambda_re, A_Lambda_im, A_B_re, A_B_im, A_C_re, A_C_im, A_log_dt, A_Dskip,
    B_x, B_w1, B_w2, B_w3, B_w4,
):
    x2 = A_x.reshape(L, D)
    out = pl.pallas_call(
        _kernel,
        grid=(NB + 1,),
        in_specs=[pl.BlockSpec(memory_space=pl.ANY)] * 13,
        out_specs=pl.BlockSpec(memory_space=pl.ANY),
        out_shape=jax.ShapeDtypeStruct((L, D), f32),
        scratch_shapes=[
            pltpu.VMEM((D, 2 * P), bf16),
            pltpu.VMEM((8, 8, P), f32),
            pltpu.VMEM((2, 8, P), f32),
            pltpu.VMEM((2 * NT, UR, 128), f32),
            pltpu.VMEM((2 * NT, UR, 128), f32),
            pltpu.VMEM((2 * NT, UR, 128), f32),
            pltpu.VMEM((3, TM + 2 * HALO, D), f32),
            pltpu.VMEM((4, TM, D), bf16),
            pltpu.VMEM((3, TM, D), f32),
            pltpu.VMEM((2 * P, D), bf16),
            pltpu.VMEM((D, P), bf16), pltpu.VMEM((D, P), bf16),
            pltpu.VMEM((D, D), bf16), pltpu.VMEM((D, D), bf16),
            pltpu.VMEM((D, F), bf16), pltpu.VMEM((F, D), bf16),
            pltpu.VMEM((L, D), bf16),
            pltpu.VMEM((P,), bf16), pltpu.VMEM((P,), bf16),
            pltpu.VMEM((P,), bf16), pltpu.VMEM((D,), bf16),
            pltpu.SemaphoreType.DMA((12,)),
            pltpu.SemaphoreType.DMA((NB,)),
            pltpu.VMEM((TM, D), bf16),
            pltpu.VMEM((TM, D), bf16),
            pltpu.VMEM((TM, D), f32),
            pltpu.VMEM((2 * NT, UR, 128), f32),
            pltpu.VMEM((2, TM, D), f32),
            pltpu.SemaphoreType.DMA((4,)),
        ],
        compiler_params=pltpu.CompilerParams(
            dimension_semantics=("arbitrary",),
            vmem_limit_bytes=100 * 1024 * 1024,
        ),
    )(x2, A_Lambda_re, A_Lambda_im, A_log_dt, A_Dskip,
      A_B_re, A_B_im, A_C_re, A_C_im, B_w1, B_w2, B_w3, B_w4)
    return out.reshape(1, L, D)
```
